```python
import os as _os
_os.environ.setdefault("JAX_PLATFORMS", "cpu")
import jax
import jax.numpy as jnp

def _softmax(x, axis=-1):
    return jax.nn.softmax(x, axis=axis)
def _gelu(x):
    return jax.nn.gelu(x, approximate=True)
def _silu(x):
    return jax.nn.silu(x)
def _sigmoid(x):
    return jax.nn.sigmoid(x)
def _layernorm(x, axis=-1, eps=1e-5):
    m = jnp.mean(x, axis=axis, keepdims=True)
    v = jnp.var(x, axis=axis, keepdims=True)
    return (x - m) / jnp.sqrt(v + eps)
def _scatter_add(tgt, idx, src, axis=0):
    return tgt.at[idx].add(src)
def _segment_sum(src, seg, n):
    return jax.ops.segment_sum(src, seg, n)
class _Rng:
    def __init__(self, key):
        self._k = key
    def _next(self):
        self._k, sub = jax.random.split(self._k)
        return sub
    def normal(self, shape):
        return jax.random.normal(self._next(), shape, dtype=jnp.bfloat16)
    def randint(self, lo, hi, shape):
        return jax.random.randint(self._next(), shape, lo, hi, dtype=jnp.int32)
    def uniform(self, shape, lo=0.0, hi=1.0):
        return jax.random.uniform(self._next(), shape, jnp.bfloat16, lo, hi)
    def permutation(self, n):
        return jax.random.permutation(self._next(), n)


kernel_name = 'interleave_layers__sliding_block_cached__mixer_channel_mlp__decode'

def setup_inputs():
    _rng = _Rng(jax.random.key(int.from_bytes(__import__("os").urandom(4), "little")))
    _w = (lambda a: (lambda t: t.astype(jnp.bfloat16) if jnp.issubdtype(t.dtype, jnp.floating) else t)(jnp.asarray(a)))
    def _A_setup():
        B, Sq, D = 8, 1, 1024
        Hq, Hkv, Sk, Dh = 32, 4, 4096, 128
        assert Hq % Hkv == 0, (Hq, Hkv)
        return {
            "x": _w((lambda *s: _rng.normal(s) * 0.05)(B, Sq, D)),
            "k_cache": _w((lambda *s: _rng.normal(s) * 1.6)(B, Hkv, Sk, Dh)),
            "v_cache": _w((lambda *s: _rng.normal(s) * 0.8)(B, Hkv, Sk, Dh)),
            "wq": _w((lambda *s: _rng.normal(s) * 1.6)(D, Hq * Dh) * (D ** -0.5)),
            "wo": _w((lambda *s: _rng.normal(s) * 0.8)(Hq * Dh, D) * ((Hq * Dh) ** -0.5)),
        }
    _A_in = _A_setup()

    def _B_setup():
        B, S, D, F = 8, 1, 1024, 3584
        return {
            "x": _w((lambda *s: _rng.normal(s) * 0.05)(B, S, D)),
            "w1": _w((lambda *s: _rng.normal(s) * 0.4)(D, F) * (D ** -0.5)),
            "b1": _w((lambda *s: _rng.normal(s) * 0.4)(F)),
            "w2": _w((lambda *s: _rng.normal(s) * 0.4)(F, D) * (F ** -0.5)),
            "b2": _w((lambda *s: _rng.normal(s) * 0.1)(D)),
        }
    _B_in = _B_setup()

    return {
        "A_x": _A_in["x"],
        "A_k_cache": _A_in["k_cache"],
        "A_v_cache": _A_in["v_cache"],
        "A_wq": _A_in["wq"],
        "A_wo": _A_in["wo"],
        "B_x": _B_in["x"],
        "B_w1": _B_in["w1"],
        "B_b1": _B_in["b1"],
        "B_w2": _B_in["w2"],
        "B_b2": _B_in["b2"],
    }

def reference(A_x, A_k_cache, A_v_cache, A_wq, A_wo, B_x, B_w1, B_b1, B_w2, B_b2):
    def _A_ref(x, k_cache, v_cache, wq, wo):
        B, Sq, D = x.shape
        Hq, Dh = 32, 128
        Hkv, Sk = k_cache.shape[1], k_cache.shape[2]
        W = min(4096, max(256, Sk // 4))
        rep = Hq // Hkv
        q = (lambda x, *d: x.transpose(*d))((x @ wq).reshape(B, Sq, Hq, Dh), 0, 2, 1, 3)
        k = jnp.repeat(k_cache[:, :, Sk - W:, :], rep, axis=1)
        v = jnp.repeat(v_cache[:, :, Sk - W:, :], rep, axis=1)
        scores = jnp.einsum("bhqd,bhkd->bhqk", q, k) * (Dh ** -0.5)
        p = _softmax(scores, axis=-1)
        o = jnp.einsum("bhqk,bhkd->bhqd", p, v)
        return (lambda x, *d: x.transpose(*d))(o, 0, 2, 1, 3).reshape(B, Sq, Hq * Dh) @ wo

    def _B_ref(x, w1, b1, w2, b2):
        y = _layernorm(x, axis=-1)
        h = _gelu(jnp.einsum("bsd,df->bsf", y, w1) + b1)
        return jnp.einsum("bsf,fd->bsd", h, w2) + b2

    x = A_x
    x = x + _A_ref(_layernorm(x, axis=-1), A_k_cache, A_v_cache, A_wq, A_wo)
    x = x + _B_ref(_layernorm(x, axis=-1), B_w1, B_b1, B_w2, B_b2)
    x = x + _A_ref(_layernorm(x, axis=-1), A_k_cache, A_v_cache, A_wq, A_wo)
    x = x + _B_ref(_layernorm(x, axis=-1), B_w1, B_b1, B_w2, B_b2)
    return x
```

```python
import jax
import jax.numpy as jnp
from jax import lax
import jax.experimental.pallas as pl
import jax.experimental.pallas.tpu as pltpu

F32 = jnp.float32
BF16 = jnp.bfloat16
T = 128
LN_EPS = 1e-5


def _ln(x):
    m = jnp.mean(x, axis=-1, keepdims=True)
    xc = x - m
    v = jnp.mean(xc * xc, axis=-1, keepdims=True)
    return xc * lax.rsqrt(v + LN_EPS)


def _gelu(x):
    c = 0.7978845608028654
    return 0.5 * x * (1.0 + jnp.tanh(c * (x + 0.044715 * (x * x * x))))


def _mm(lhs_tiles, w_ref, n0, n1):
    acc = None
    for k, a in lhs_tiles:
        y = jnp.dot(a, w_ref[k * T:(k + 1) * T, n0:n1], preferred_element_type=F32)
        acc = y if acc is None else acc + y
    return acc


def _tiles(x):
    return [(k, x[:, k * T:(k + 1) * T]) for k in range(x.shape[1] // T)]


def _kernel(x_hbm, k_hbm, v_hbm, wq_hbm, wo_hbm, w1_hbm, b1_hbm, w2_hbm, b2_hbm, o_ref,
            xs, b1s, b2s, ks, kts, vs, wqs, wos, w1s, w2s, rel, ps, sems):
    B, Hkv, W, Dh = ks.shape
    Sk = k_hbm.shape[2]
    D, HD = wqs.shape
    Fd = w1s.shape[1]
    rep = HD // Dh // Hkv
    scale = Dh ** -0.5
    NB = 4 * T

    srcs = [x_hbm, wq_hbm, b1_hbm, b2_hbm,
            k_hbm.at[:, :, pl.ds(Sk - W, W), :], v_hbm.at[:, :, pl.ds(Sk - W, W), :],
            wo_hbm, w1_hbm]
    dsts = [xs, wqs, b1s, b2s, ks, vs, wos, w1s]
    F0 = Fd - 4 * T
    srcs += [w2_hbm.at[pl.ds(0, F0)], w2_hbm.at[pl.ds(F0, Fd - F0)]]
    dsts += [w2s.at[pl.ds(0, F0)], w2s.at[pl.ds(F0, Fd - F0)]]
    cps = [pltpu.make_async_copy(s, d, sems.at[i]) for i, (s, d) in enumerate(zip(srcs, dsts))]
    for c in cps:
        c.start()
    c_x, c_wq, c_b1, c_b2, c_k, c_v, c_wo, c_w1, c_w2a, c_w2b = cps

    def attn(x, first):
        xt = _tiles(_ln(x).astype(BF16))
        if first:
            c_wq.wait()
        for n in range(0, HD, NB):
            q = _mm(xt, wqs, n, n + NB)
            for j in range(NB // T):
                h = n // T + j
                rel[h * B:(h + 1) * B, :] = q[:, j * T:(j + 1) * T]
        if first:
            c_k.wait()
            for b in range(B):
                for g in range(Hkv):
                    kts[b, g] = ks[b, g].T
        inv = {}
        for g in range(Hkv):
            for b in range(B):
                q = rel[pl.ds(g * rep * B + b, rep, stride=B), :].astype(BF16)
                s = jnp.dot(q, kts[b, g], preferred_element_type=F32) * scale
                p = jnp.exp(s - jnp.max(s, axis=-1, keepdims=True))
                inv[g, b] = 1.0 / jnp.sum(p, axis=-1, keepdims=True)
                ps[g * B + b] = p
        if first:
            c_v.wait()
        for g in range(Hkv):
            for b in range(B):
                o = jnp.dot(ps[g * B + b].astype(BF16), vs[b, g], preferred_element_type=F32)
                rel[pl.ds(g * rep * B + b, rep, stride=B), :] = o * inv[g, b]
        ot = [(h, rel[h * B:(h + 1) * B, :].astype(BF16)) for h in range(HD // T)]
        if first:
            c_wo.wait()
        y = jnp.concatenate([_mm(ot, wos, n, n + NB) for n in range(0, D, NB)], axis=1)
        return x + y

    def mlp(x, first, b1, b2):
        yt = _tiles(_ln(_ln(x)).astype(BF16))
        if first:
            c_w1.wait()
        ht = []
        for n in range(0, Fd, NB):
            h = _gelu(_mm(yt, w1s, n, n + NB) + b1[:, n:n + NB]).astype(BF16)
            ht += [(n // T + j, h[:, j * T:(j + 1) * T]) for j in range(NB // T)]
        if first:
            c_w2a.wait()
        ya = [_mm(ht[:F0 // T], w2s, n, n + NB) for n in range(0, D, NB)]
        if first:
            c_w2b.wait()
        yb = [_mm(ht[F0 // T:], w2s, n, n + NB) for n in range(0, D, NB)]
        y = jnp.concatenate([a + b for a, b in zip(ya, yb)], axis=1)
        return x + (y + b2)

    def row(ref):
        v = ref[...].astype(F32)
        return jnp.concatenate(
            [jnp.broadcast_to(v[j:j + 1, :], (B, T)) for j in range(v.shape[0])], axis=1)

    c_x.wait()
    x = xs[...].astype(F32)
    x = attn(x, True)
    c_b1.wait()
    c_b2.wait()
    b1 = row(b1s)
    b2 = row(b2s)
    x = mlp(x, True, b1, b2)
    x = attn(x, False)
    x = mlp(x, False, b1, b2)
    o_ref[...] = x.astype(o_ref.dtype)


@jax.jit
def pallas_interleave_layers__sliding_block_cached__mixer_channel_mlp__decode_kernel(
    A_x: jax.Array,
    A_k_cache: jax.Array,
    A_v_cache: jax.Array,
    A_wq: jax.Array,
    A_wo: jax.Array,
    B_x: jax.Array,
    B_w1: jax.Array,
    B_b1: jax.Array,
    B_w2: jax.Array,
    B_b2: jax.Array,
):
    del B_x
    B, Sq, D = A_x.shape
    _, Hkv, Sk, Dh = A_k_cache.shape
    HD = A_wq.shape[1]
    Fd = B_w1.shape[1]
    W = min(4096, max(256, Sk // 4))
    dt = A_x.dtype
    any_ = pl.BlockSpec(memory_space=pl.ANY)
    out = pl.pallas_call(
        _kernel,
        out_shape=jax.ShapeDtypeStruct((B, D), dt),
        in_specs=[any_] * 9,
        out_specs=pl.BlockSpec(memory_space=pltpu.VMEM),
        scratch_shapes=[
            pltpu.VMEM((B, D), dt),
            pltpu.VMEM((Fd // T, T), dt),
            pltpu.VMEM((D // T, T), dt),
            pltpu.VMEM((B, Hkv, W, Dh), dt),
            pltpu.VMEM((B, Hkv, Dh, W), dt),
            pltpu.VMEM((B, Hkv, W, Dh), dt),
            pltpu.VMEM((D, HD), dt),
            pltpu.VMEM((HD, D), dt),
            pltpu.VMEM((D, Fd), dt),
            pltpu.VMEM((Fd, D), dt),
            pltpu.VMEM((HD // T * B, T), F32),
            pltpu.VMEM((Hkv * B, HD // Dh // Hkv, W), F32),
            pltpu.SemaphoreType.DMA((10,)),
        ],
        compiler_params=pltpu.CompilerParams(vmem_limit_bytes=100 * 1024 * 1024),
        name="interleave_decode",
    )(A_x.reshape(B, D), A_k_cache, A_v_cache, A_wq, A_wo, B_w1,
      B_b1.reshape(Fd // T, T), B_w2, B_b2.reshape(D // T, T))
    return out.reshape(B, Sq, D)
```

```python
import jax
import jax.numpy as jnp
from jax import lax
import jax.experimental.pallas as pl
import jax.experimental.pallas.tpu as pltpu

F32 = jnp.float32
BF16 = jnp.bfloat16
T = 128
NB = 4 * T
LN_EPS = 1e-5
LOG2E = 1.4426950408889634
CFG = dict(stages=(((17, 0, 0, 4),), ((17, 4, 4, 7),), ((4, 0, 4, 7),), ((17, 4, 7, 8),), ((4, 0, 7, 8),)),
           w1first=2, outf32=False, lag=4, merge=True)


def _sum(x):
    return jnp.sum(x, axis=-1, keepdims=True)


def _mean(x):
    return jnp.mean(x, axis=-1, keepdims=True)


def _ln_stats(x):
    m = _mean(x)
    d = x - m
    return m, d, lax.rsqrt(_mean(d * d) + LN_EPS)


def _ln(x):
    _, d, r = _ln_stats(x)
    return d * r


def _gelu(x):
    c = 0.7978845608028654
    return 0.5 * x * (1.0 + jnp.tanh(c * (x + 0.044715 * (x * x * x))))


def _mm(lhs_tiles, w_ref, n0, n1, acc=None):
    for k, a in lhs_tiles:
        y = jnp.dot(a, w_ref[k * T:(k + 1) * T, n0:n1], preferred_element_type=F32)
        acc = y if acc is None else acc + y
    return acc


def _tiles(x, k0=0):
    return [(k0 + k, x[:, k * T:(k + 1) * T].astype(BF16)) for k in range(x.shape[1] // T)]


def _kernel(x_hbm, k_hbm, v_hbm, wq_hbm, wo_hbm, w1_hbm, b1_hbm, w2_hbm, b2_hbm, o_ref,
            xs, b1s, b2s, ks, kts, vs, wqs, wos, w1s, w2s, qs, os_, csq, cs1, b1b, last_sem):
    B, Hkv, W, Dh = ks.shape
    Sk = k_hbm.shape[2]
    D, HD = wqs.shape
    Fd = w1s.shape[1]
    rep = HD // Dh // Hkv
    qscale = Dh ** -0.5 * LOG2E
    nF, nD = Fd // T, D // T
    stages = [[(nF - a, nF - b, c0, c1) for a, b, c0, c1 in st] for st in CFG["stages"]]
    stages = [[(0, min(p[0] for st in stages for p in st), 0, nD)]] + stages

    def with_ones(y):
        return jnp.concatenate([y, jnp.ones_like(y)], axis=0)

    def put_q(q, n):
        for j in range(q.shape[1] // T):
            h = n // T + j
            qs[h * B:(h + 1) * B, :] = q[:, j * T:(j + 1) * T]

    def attend():
        units = [(g, b) for g in range(Hkv) for b in range(B)]
        lag, probs = CFG["lag"], {}
        for i in range(len(units) + lag):
            if i < len(units):
                g, b = units[i]
                q = qs[pl.ds(g * rep * B + b, rep, stride=B), :].astype(BF16)
                s = jnp.dot(q, kts[b, g], preferred_element_type=F32)
                p = jnp.exp2(s - jnp.max(s, axis=-1, keepdims=True))
                probs[i] = (p.astype(BF16), 1.0 / _sum(p))
            if i >= lag:
                g, b = units[i - lag]
                p, inv = probs.pop(i - lag)
                o = jnp.dot(p, vs[b, g], preferred_element_type=F32)
                os_[pl.ds(g * rep * B + b, rep, stride=B), :] = o * inv
        return [(h, os_[h * B:(h + 1) * B, :].astype(BF16)) for h in range(HD // T)]

    def row(ref):
        v = ref[...].astype(F32)
        return jnp.concatenate(
            [jnp.broadcast_to(v[j:j + 1, :], (B, T)) for j in range(v.shape[0])], axis=1)

    def w2_copies(stage, sem):
        idx = [(pl.ds(r0 * T, (r1 - r0) * T), pl.ds(c0 * T, (c1 - c0) * T)) for r0, r1, c0, c1 in stage]
        return [pltpu.make_async_copy(w2_hbm.at[i], w2s.at[i], sem) for i in idx]

    def wait(group):
        for c in group:
            c.wait()

    left = [nF] * nD

    def w2_stage(stage, ht, acc, qraw):
        acc = list(acc)
        done = []
        for r0, r1, c0, c1 in stage:
            for c in range(c0, c1, 4):
                e = min(c + 4, c1)
                y = _mm(ht[r0:r1], w2s, c * T, e * T)
                for j in range(c, e):
                    acc[j] = acc[j] + y[:, (j - c) * T:(j - c + 1) * T]
                    left[j] -= r1 - r0
                    if left[j] == 0:
                        done.append((j, acc[j].astype(BF16)))
        if done:
            qraw = [_mm(done, wqs, i * NB, (i + 1) * NB, a) for i, a in enumerate(qraw)]
        return acc, qraw

    g_last = w2_copies(stages[-1], last_sem)

    def first_pass(sems):
        win = pl.ds(Sk - W, W)
        pairs = [[(wq_hbm, wqs), (x_hbm, xs), (b1_hbm, b1s), (b2_hbm, b2s)],
                 [(k_hbm.at[:, :, win, :], ks), (v_hbm.at[:, :, win, :], vs)],
                 [(wo_hbm, wos)], [(w1_hbm, w1s)]]
        groups = [[pltpu.make_async_copy(s, d, sems.at[i]) for s, d in p] for i, p in enumerate(pairs)]
        groups += [w2_copies(st, sems.at[len(pairs) + i]) for i, st in enumerate(stages[:-1])]
        for grp in groups + [g_last]:
            for c in grp:
                c.start()

        wait(groups[0])
        x0 = xs[...].astype(F32)
        xt = _tiles(with_ones(_ln(x0)))
        for n in range(0, HD, NB):
            y = _mm(xt, wqs, n, n + NB)
            put_q(y[:B] * qscale, n)
            csq[:, n:n + NB] = y[B:]
        b1b[...] = row(b1s)
        b2 = row(b2s)
        wait(groups[1])
        for b in range(B):
            for g in range(Hkv):
                kts[b, g] = ks[b, g].T
        ot = attend()
        wait(groups[2])
        x1 = x0 + jnp.concatenate([_mm(ot, wos, n, n + NB) for n in range(0, D, NB)], axis=1)

        yt = _tiles(with_ones(_ln(_ln(x1))))
        base = x1 + b2
        shift = _mean(base)
        base = base - shift
        wait(groups[3])
        ht = []
        for n in range(0, Fd, NB):
            y = _mm(yt, w1s, n, n + NB)
            cs1[:, n:n + NB] = y[B:]
            ht += _tiles(_gelu(y[:B] + b1b[:, n:n + NB]), n // T)
        acc = [base[:, j * T:(j + 1) * T] for j in range(nD)]
        qraw = [None] * (HD // NB)
        for grp, st in zip(groups[4:], stages[:-1]):
            wait(grp)
            acc, qraw = w2_stage(st, ht, acc, qraw)
        return [h for _, h in ht], acc, qraw, shift, b2

    ht, acc, qraw, shift, b2 = pl.run_scoped(first_pass, pltpu.SemaphoreType.DMA((3 + len(stages),)))
    ht = list(enumerate(ht))
    early = [j for j in range(nD) if left[j] == 0]
    late = [j for j in range(nD) if left[j] != 0]
    if early:
        xe = jnp.concatenate([acc[j] for j in early], axis=1)
        mu = _mean(xe)
        m2e = _sum((xe - mu) * (xe - mu))
    wait(g_last)
    acc, qraw = w2_stage(stages[-1], ht, acc, qraw)

    xc = jnp.concatenate(acc, axis=1)
    if early:
        dl = jnp.concatenate([acc[j] for j in late], axis=1) - mu
        s1, s2 = _sum(dl), _sum(dl * dl)
        m = mu + s1 * (1.0 / D)
        r = lax.rsqrt((m2e + (s2 - s1 * s1 * (1.0 / D))) * (1.0 / D) + LN_EPS)
        d2 = xc - m
    else:
        m, d2, r = _ln_stats(xc)
    shift = shift + m
    r = r * qscale
    for i, a in enumerate(qraw):
        put_q(r * (a - m * csq[:, i * NB:(i + 1) * NB]), i * NB)
    ot = attend()
    xc = [d2[:, n:n + NB] + _mm(ot, wos, n, n + NB) for n in range(0, D, NB)]

    yt = [_tiles(c, i * NB // T) for i, c in enumerate(xc)]
    xc = jnp.concatenate(xc, axis=1)
    m1, d, r1 = _ln_stats(xc)
    m2, _, r2 = _ln_stats(d * r1)
    ca, cb = r1 * r2, (m1 * r1 + m2) * r2
    nfirst = CFG["w1first"]
    part = [_mm(yt[0], w1s, i * NB, (i + 1) * NB) for i in range(nfirst)]
    ht = []
    for i, n in enumerate(range(0, Fd, NB)):
        if i < nfirst:
            y = _mm(yt[1], w1s, n, n + NB, part[i])
        else:
            y = _mm(yt[0] + yt[1], w1s, n, n + NB)
        y = ca * y + (b1b[:, n:n + NB] - cb * cs1[:, n:n + NB])
        ht += _tiles(_gelu(y), n // T)
    base = xc + (shift + b2)
    for n in range(0, D, NB):
        o_ref[:, n:n + NB] = _mm(ht, w2s, n, n + NB, base[:, n:n + NB]).astype(o_ref.dtype)


@jax.jit
def pallas_interleave_layers__sliding_block_cached__mixer_channel_mlp__decode_kernel(
    A_x, A_k_cache, A_v_cache, A_wq, A_wo, B_x, B_w1, B_b1, B_w2, B_b2,
):
    del B_x
    B, Sq, D = A_x.shape
    _, Hkv, Sk, Dh = A_k_cache.shape
    HD = A_wq.shape[1]
    Fd = B_w1.shape[1]
    W = min(4096, max(256, Sk // 4))
    dt = A_x.dtype
    any_ = pl.BlockSpec(memory_space=pl.ANY)
    out = pl.pallas_call(
        _kernel,
        out_shape=jax.ShapeDtypeStruct((B, D), F32 if CFG["outf32"] else dt),
        in_specs=[any_] * 9,
        out_specs=pl.BlockSpec(memory_space=pltpu.VMEM),
        scratch_shapes=[
            pltpu.VMEM((B, D), dt),
            pltpu.VMEM((Fd // T, T), dt),
            pltpu.VMEM((D // T, T), dt),
            pltpu.VMEM((B, Hkv, W, Dh), dt),
            pltpu.VMEM((B, Hkv, Dh, W), dt),
            pltpu.VMEM((B, Hkv, W, Dh), dt),
            pltpu.VMEM((D, HD), dt),
            pltpu.VMEM((HD, D), dt),
            pltpu.VMEM((D, Fd), dt),
            pltpu.VMEM((Fd, D), dt),
            pltpu.VMEM((HD // T * B, T), F32),
            pltpu.VMEM((HD // T * B, T), F32),
            pltpu.VMEM((B, HD), F32),
            pltpu.VMEM((B, Fd), F32),
            pltpu.VMEM((B, Fd), F32),
            pltpu.SemaphoreType.DMA(()),
        ],
        compiler_params=pltpu.CompilerParams(vmem_limit_bytes=100 * 1024 * 1024),
        name="interleave_decode",
    )(A_x.reshape(B, D), A_k_cache, A_v_cache, A_wq, A_wo, B_w1,
      B_b1.reshape(Fd // T, T), B_w2, B_b2.reshape(D // T, T))
    return out.reshape(B, Sq, D).astype(dt)
```

```python
import jax
import jax.numpy as jnp
from jax import lax
import jax.experimental.pallas as pl
import jax.experimental.pallas.tpu as pltpu

F32 = jnp.float32
BF16 = jnp.bfloat16
T = 128
NB = 4 * T
LN_EPS = 1e-5
LOG2E = 1.4426950408889634
TAIL_ROWS = 13
W2_PIECES = ((13, 4, 0, 5), (4, 0, 0, 5), (13, 0, 5, 7))
HELD_BLOCKS = 1
PV_LAG = 4
W1_EARLY = 2


def _sum(x):
    return jnp.sum(x, axis=-1, keepdims=True)


def _mean(x):
    return jnp.mean(x, axis=-1, keepdims=True)


def _ln_stats(x):
    m = _mean(x)
    d = x - m
    return m, d, lax.rsqrt(_mean(d * d) + LN_EPS)


def _ln(x):
    _, d, r = _ln_stats(x)
    return d * r


def _gelu(x):
    c = 0.7978845608028654
    return 0.5 * x * (1.0 + jnp.tanh(c * (x + 0.044715 * (x * x * x))))


def _mm(lhs_tiles, rhs_tile, acc=None):
    for k, a in lhs_tiles:
        y = jnp.dot(a, rhs_tile(k), preferred_element_type=F32)
        acc = y if acc is None else acc + y
    return acc


def _cols(w_ref, n):
    return lambda k: w_ref[k * T:(k + 1) * T, n:n + NB]


def _tiles(x, k0=0):
    return [(k0 + k, x[:, k * T:(k + 1) * T].astype(BF16)) for k in range(x.shape[1] // T)]


def _kernel(x_hbm, k_hbm, v_hbm, wq_hbm, wo_hbm, w1_hbm, b1_hbm, w2_hbm, b2_hbm, o_ref,
            xs, b1s, b2s, ks, kts, vs, wqs, wos, w1s, w2s, w2e, qs, os_, csq, cs1, b1b, last_sem):
    B, Hkv, W, Dh = ks.shape
    Sk = k_hbm.shape[2]
    D, HD = wqs.shape
    Fd = w1s.shape[1]
    rep = HD // Dh // Hkv
    qscale = Dh ** -0.5 * LOG2E
    nF, nD, nQ = Fd // T, D // T, HD // NB
    e0 = nF - w2e.shape[0] // T
    pieces = [(0, e0, 0, nD)] + [(nF - a, nF - b, c0, c1) for a, b, c0, c1 in W2_PIECES]

    def w2_cols(c0, c1):
        def tile(k):
            rows = slice(k * T, (k + 1) * T)
            if k < e0 or c1 < nD:
                return w2s[rows, c0 * T:c1 * T]
            e = w2e[(k - e0) * T:(k - e0 + 1) * T, :]
            return e if c0 == nD - 1 else jnp.concatenate([w2s[rows, c0 * T:(c1 - 1) * T], e], axis=1)
        return tile

    def with_ones(y):
        return jnp.concatenate([y, jnp.ones_like(y)], axis=0)

    def put_q(q, n):
        for j in range(q.shape[1] // T):
            h = n // T + j
            qs[h * B:(h + 1) * B, :] = q[:, j * T:(j + 1) * T]

    def attend():
        units = [(g, b) for g in range(Hkv) for b in range(B)]
        probs = {}
        for i in range(len(units) + PV_LAG):
            if i < len(units):
                g, b = units[i]
                q = qs[pl.ds(g * rep * B + b, rep, stride=B), :].astype(BF16)
                s = jnp.dot(q, kts[b, g], preferred_element_type=F32)
                p = jnp.exp2(s - jnp.max(s, axis=-1, keepdims=True))
                probs[i] = (p.astype(BF16), 1.0 / _sum(p))
            if i >= PV_LAG:
                g, b = units[i - PV_LAG]
                p, inv = probs.pop(i - PV_LAG)
                o = jnp.dot(p, vs[b, g], preferred_element_type=F32)
                os_[pl.ds(g * rep * B + b, rep, stride=B), :] = o * inv
        return [(h, os_[h * B:(h + 1) * B, :].astype(BF16)) for h in range(HD // T)]

    def bias_rows(ref):
        v = ref[...].astype(F32)
        return jnp.concatenate(
            [jnp.broadcast_to(v[j:j + 1, :], (B, T)) for j in range(v.shape[0])], axis=1)

    def project_q(qraw, blocks, acc, cols):
        lhs = [(j, acc[j].astype(BF16)) for j in cols]
        for i in blocks:
            qraw[i] = _mm(lhs, _cols(wqs, i * NB), qraw[i])

    last = pltpu.make_async_copy(
        w2_hbm.at[pl.ds(e0 * T, (nF - e0) * T), pl.ds((nD - 1) * T, T)], w2e, last_sem)
    held = range(nQ - HELD_BLOCKS, nQ)
    held_cols = range(pieces[-1][2], pieces[-1][3])

    def first_pair(sems):
        win = pl.ds(Sk - W, W)
        pairs = [[(wq_hbm, wqs), (x_hbm, xs), (b1_hbm, b1s), (b2_hbm, b2s)],
                 [(k_hbm.at[:, :, win, :], ks), (v_hbm.at[:, :, win, :], vs)],
                 [(wo_hbm, wos)], [(w1_hbm, w1s)]]
        for r0, r1, c0, c1 in pieces:
            idx = (pl.ds(r0 * T, (r1 - r0) * T), pl.ds(c0 * T, (c1 - c0) * T))
            pairs.append([(w2_hbm.at[idx], w2s.at[idx])])
        groups = [[pltpu.make_async_copy(s, d, sems.at[i]) for s, d in p]
                  for i, p in enumerate(pairs)]
        for group in groups:
            for c in group:
                c.start()
        last.start()

        def wait(i):
            for c in groups[i]:
                c.wait()

        wait(0)
        x0 = xs[...].astype(F32)
        xt = _tiles(with_ones(_ln(x0)))
        for n in range(0, HD, NB):
            y = _mm(xt, _cols(wqs, n))
            put_q(y[:B] * qscale, n)
            csq[:, n:n + NB] = y[B:]
        b1b[...] = bias_rows(b1s)
        b2 = bias_rows(b2s)
        wait(1)
        for b in range(B):
            for g in range(Hkv):
                kts[b, g] = ks[b, g].T
        ot = attend()
        wait(2)
        x1 = x0 + jnp.concatenate([_mm(ot, _cols(wos, n)) for n in range(0, D, NB)], axis=1)

        yt = _tiles(with_ones(_ln(_ln(x1))))
        base = x1 + b2
        shift = _mean(base)
        base = base - shift
        wait(3)
        ht = []
        for n in range(0, Fd, NB):
            y = _mm(yt, _cols(w1s, n))
            cs1[:, n:n + NB] = y[B:]
            ht += _tiles(_gelu(y[:B] + b1b[:, n:n + NB]), n // T)
        acc = [base[:, j * T:(j + 1) * T] for j in range(nD)]
        left = [nF] * nD
        qraw = [None] * nQ
        for i, (r0, r1, c0, c1) in enumerate(pieces):
            wait(4 + i)
            for c in range(c0, c1, 4):
                e = min(c + 4, c1)
                y = _mm(ht[r0:r1], w2_cols(c, e))
                for j in range(c, e):
                    acc[j] = acc[j] + y[:, (j - c) * T:(j - c + 1) * T]
                    left[j] -= r1 - r0
            done = [j for j in range(c0, c1) if left[j] == 0]
            if done:
                project_q(qraw, range(held[0] if i == len(pieces) - 1 else nQ), acc, done)
        assert left == [0] * (nD - 1) + [nF - e0]
        xe = jnp.concatenate(acc[:-1], axis=1)
        mu = _mean(xe)
        return [h for _, h in ht], acc, qraw, shift, b2, mu, _sum((xe - mu) * (xe - mu))

    ht, acc, qraw, shift, b2, mu, ssq = pl.run_scoped(
        first_pair, pltpu.SemaphoreType.DMA((4 + len(pieces),)))
    last.wait()
    acc[-1] = acc[-1] + _mm(list(enumerate(ht))[e0:], w2_cols(nD - 1, nD))
    project_q(qraw, held, acc, held_cols)
    project_q(qraw, range(nQ), acc, [nD - 1])

    dl = acc[-1] - mu
    s1, s2 = _sum(dl), _sum(dl * dl)
    m = mu + s1 * (1.0 / D)
    r = lax.rsqrt((ssq + (s2 - s1 * s1 * (1.0 / D))) * (1.0 / D) + LN_EPS) * qscale
    for i, a in enumerate(qraw):
        put_q(r * (a - m * csq[:, i * NB:(i + 1) * NB]), i * NB)
    x2 = jnp.concatenate(acc, axis=1) - m
    shift = shift + m
    ot = attend()
    x3 = [x2[:, n:n + NB] + _mm(ot, _cols(wos, n)) for n in range(0, D, NB)]

    yt = [_tiles(c, i * NB // T) for i, c in enumerate(x3)]
    x3 = jnp.concatenate(x3, axis=1)
    m1, d, r1 = _ln_stats(x3)
    m2, _, r2 = _ln_stats(d * r1)
    ca, cb = r1 * r2, (m1 * r1 + m2) * r2
    early = [_mm(yt[0], _cols(w1s, i * NB)) for i in range(W1_EARLY)]
    rest = [t for c in yt[1:] for t in c]
    ht = []
    for i, n in enumerate(range(0, Fd, NB)):
        if i < len(early):
            y = _mm(rest, _cols(w1s, n), early[i])
        else:
            y = _mm(yt[0] + rest, _cols(w1s, n))
        y = ca * y + (b1b[:, n:n + NB] - cb * cs1[:, n:n + NB])
        ht += _tiles(_gelu(y), n // T)
    base = x3 + (shift + b2)
    for c in range(0, nD, 4):
        y = _mm(ht, w2_cols(c, c + 4), base[:, c * T:c * T + NB])
        o_ref[:, c * T:c * T + NB] = y.astype(o_ref.dtype)


@jax.jit
def pallas_interleave_layers__sliding_block_cached__mixer_channel_mlp__decode_kernel(
    A_x: jax.Array,
    A_k_cache: jax.Array,
    A_v_cache: jax.Array,
    A_wq: jax.Array,
    A_wo: jax.Array,
    B_x: jax.Array,
    B_w1: jax.Array,
    B_b1: jax.Array,
    B_w2: jax.Array,
    B_b2: jax.Array,
):
    del B_x
    B, Sq, D = A_x.shape
    _, Hkv, Sk, Dh = A_k_cache.shape
    HD = A_wq.shape[1]
    Fd = B_w1.shape[1]
    W = min(4096, max(256, Sk // 4))
    dt = A_x.dtype
    out = pl.pallas_call(
        _kernel,
        out_shape=jax.ShapeDtypeStruct((B, D), dt),
        in_specs=[pl.BlockSpec(memory_space=pl.ANY)] * 9,
        out_specs=pl.BlockSpec(memory_space=pltpu.VMEM),
        scratch_shapes=[
            pltpu.VMEM((B, D), dt),
            pltpu.VMEM((Fd // T, T), dt),
            pltpu.VMEM((D // T, T), dt),
            pltpu.VMEM((B, Hkv, W, Dh), dt),
            pltpu.VMEM((B, Hkv, Dh, W), dt),
            pltpu.VMEM((B, Hkv, W, Dh), dt),
            pltpu.VMEM((D, HD), dt),
            pltpu.VMEM((HD, D), dt),
            pltpu.VMEM((D, Fd), dt),
            pltpu.VMEM((Fd, D), dt),
            pltpu.VMEM((TAIL_ROWS * T, T), dt),
            pltpu.VMEM(((HD // T + 1) * B, T), F32),
            pltpu.VMEM(((HD // T + 1) * B, T), F32),
            pltpu.VMEM((B, HD), F32),
            pltpu.VMEM((B, Fd), F32),
            pltpu.VMEM((B, Fd), F32),
            pltpu.SemaphoreType.DMA(()),
        ],
        compiler_params=pltpu.CompilerParams(vmem_limit_bytes=100 * 1024 * 1024),
        name="interleave_decode",
    )(A_x.reshape(B, D), A_k_cache, A_v_cache, A_wq, A_wo, B_w1,
      B_b1.reshape(Fd // T, T), B_w2, B_b2.reshape(D // T, T))
    return out.reshape(B, Sq, D)
```
